```python
import os as _os
_os.environ.setdefault("JAX_PLATFORMS", "cpu")
import jax
import jax.numpy as jnp

def _softmax(x, axis=-1):
    return jax.nn.softmax(x, axis=axis)
def _gelu(x):
    return jax.nn.gelu(x, approximate=True)
def _silu(x):
    return jax.nn.silu(x)
def _sigmoid(x):
    return jax.nn.sigmoid(x)
def _layernorm(x, axis=-1, eps=1e-5):
    m = jnp.mean(x, axis=axis, keepdims=True)
    v = jnp.var(x, axis=axis, keepdims=True)
    return (x - m) / jnp.sqrt(v + eps)
def _scatter_add(tgt, idx, src, axis=0):
    return tgt.at[idx].add(src)
def _segment_sum(src, seg, n):
    return jax.ops.segment_sum(src, seg, n)
class _Rng:
    def __init__(self, key):
        self._k = key
    def _next(self):
        self._k, sub = jax.random.split(self._k)
        return sub
    def normal(self, shape):
        return jax.random.normal(self._next(), shape, dtype=jnp.bfloat16)
    def randint(self, lo, hi, shape):
        return jax.random.randint(self._next(), shape, lo, hi, dtype=jnp.int32)
    def uniform(self, shape, lo=0.0, hi=1.0):
        return jax.random.uniform(self._next(), shape, jnp.bfloat16, lo, hi)
    def permutation(self, n):
        return jax.random.permutation(self._next(), n)


kernel_name = 'gated_mix__grouped_kv_mqa__ssm_conv_s5__prompt'

def setup_inputs():
    _rng = _Rng(jax.random.key(int.from_bytes(__import__("os").urandom(4), "little")))
    _w = (lambda a: (lambda t: t.astype(jnp.bfloat16) if jnp.issubdtype(t.dtype, jnp.floating) else t)(jnp.asarray(a)))
    def _A_setup():
        B, S, D, H = 1, 2048, 512, 32
        Dh = D // H
        return {
            "x": _w((lambda *s: _rng.normal(s) * 0.05)(B, S, D)),
            "wq": _w((lambda *s: _rng.normal(s) * 1.6)(D, H * Dh)),
            "wk": _w((lambda *s: _rng.normal(s) * 1.6)(D, Dh)),
            "wv": _w((lambda *s: _rng.normal(s) * 0.05)(D, Dh)),
            "wo": _w((lambda *s: _rng.normal(s) * 0.05)(H * Dh, D)),
        }
    _A_in = _A_setup()

    def _B_setup():
        B, S, D = 1, 2048, 512
        P = D
        Lambda_re = -0.5 * jnp.exp((lambda *s: _rng.normal(s) * 0.4)(P))
        Lambda_im = (lambda *s: _rng.normal(s) * 0.4)(P) * 1.0
        B_re = (lambda *s: _rng.normal(s) * 0.4)(P, D) * (D ** -0.5)
        B_im = (lambda *s: _rng.normal(s) * 0.4)(P, D) * (D ** -0.5)
        C_re = (lambda *s: _rng.normal(s) * 0.4)(D, P) * (P ** -0.5)
        C_im = (lambda *s: _rng.normal(s) * 0.4)(D, P) * (P ** -0.5)
        log_dt = (lambda *s: _rng.normal(s) * 0.4)(P) * 0.3 - 2.0
        Dskip = (lambda *s: _rng.normal(s) * 0.4)(D)
        return {
            "x": _w((lambda *s: _rng.normal(s) * 0.05)(B, S, D)),
            "Lambda_re": _w(Lambda_re),
            "Lambda_im": _w(Lambda_im),
            "B_re": _w(B_re),
            "B_im": _w(B_im),
            "C_re": _w(C_re),
            "C_im": _w(C_im),
            "log_dt": _w(log_dt),
            "Dskip": _w(Dskip),
        }
    _B_in = _B_setup()

    return {
        "A_x": _A_in["x"],
        "A_wq": _A_in["wq"],
        "A_wk": _A_in["wk"],
        "A_wv": _A_in["wv"],
        "A_wo": _A_in["wo"],
        "B_x": _B_in["x"],
        "B_Lambda_re": _B_in["Lambda_re"],
        "B_Lambda_im": _B_in["Lambda_im"],
        "B_B_re": _B_in["B_re"],
        "B_B_im": _B_in["B_im"],
        "B_C_re": _B_in["C_re"],
        "B_C_im": _B_in["C_im"],
        "B_log_dt": _B_in["log_dt"],
        "B_Dskip": _B_in["Dskip"],
        "gate_w": _w((lambda *s: _rng.normal(s) * 0.05)(512) * 16.0),
    }

def reference(A_x, A_wq, A_wk, A_wv, A_wo, B_x, B_Lambda_re, B_Lambda_im, B_B_re, B_B_im, B_C_re, B_C_im, B_log_dt, B_Dskip, gate_w):
    def _A_ref(x, wq, wk, wv, wo):
        B, S, D = x.shape
        H = 32
        Dh = D // H
        q = (lambda x, *d: x.transpose(*d))((x @ wq).reshape(B, S, H, Dh), 0, 2, 1, 3)
        k = x @ wk
        v = x @ wv
        scores = jnp.einsum("bhqd,bkd->bhqk", q, k) * (Dh ** -0.5)
        p = _softmax(scores, axis=-1)
        o = jnp.einsum("bhqk,bkd->bhqd", p, v)
        return (lambda x, *d: x.transpose(*d))(o, 0, 2, 1, 3).reshape(B, S, H * Dh) @ wo

    def _B_ref(x, Lambda_re, Lambda_im, B_re, B_im, C_re, C_im, log_dt, Dskip):
        Bsz, L, H = x.shape
        Lam = Lambda_re + 1j * Lambda_im
        Bmat = B_re + 1j * B_im
        Cmat = C_re + 1j * C_im
        dt = jnp.exp(log_dt)
        Lam_bar = jnp.exp(dt * Lam)
        B_bar = ((Lam_bar - 1.0) / Lam)[:, None] * Bmat
        Bu = jnp.einsum("bld,pd->blp", x + 0j, B_bar)
        h = jnp.zeros_like(Bu[:, 0, :])
        hs = []
        for t in range(L):
            h = Lam_bar[None, :] * h + Bu[:, t, :]
            hs.append(h)
        hseq = jnp.stack(hs, 1)
        y = 2.0 * jnp.einsum("blp,dp->bld", hseq, Cmat).real + x * Dskip[None, None, :]
        return y

    x = A_x
    g = _sigmoid((x * gate_w).sum(-1, keepdims=True))
    a = _A_ref(x, A_wq, A_wk, A_wv, A_wo)
    b = _B_ref(x, B_Lambda_re, B_Lambda_im, B_B_re, B_B_im, B_C_re, B_C_im, B_log_dt, B_Dskip)
    return g * a + (1 - g) * b
```

```python
import jax
import jax.numpy as jnp
from jax import lax
import jax.experimental.pallas as pl
import jax.experimental.pallas.tpu as pltpu

S, D, H, DH = 2048, 512, 32, 16
DA = 2 * DH
QB, KC = 512, 128
NQB, NKC = S // QB, S // KC
NSEG, SEGL, PITCH = 16, 128, 129
LT = D // 128
HU = 4
DLY = 2
LOG2E = 1.4426950408889634
F32, BF16 = jnp.float32, jnp.bfloat16

NT = (((1,), (1,)), ((), ()))
TN = (((0,), (0,)), ((), ()))


def _dot(a, b):
    return jnp.dot(a, b, preferred_element_type=F32)


def _dg(a, b, dims):
    return lax.dot_general(a, b, dims, preferred_element_type=F32)


def _cmul(ar, ai, br, bi):
    return ar * br - ai * bi, ar * bi + ai * br


def _kernel(x_ref, wq_ref, wk_ref, wv_ref, wo_ref, lre_ref, lim_ref, bre_ref, bim_ref,
            cre_ref, cim_ref, ldt_ref, dsk_ref, gw_ref, out_ref,
            kaug, vT, wqT, qa, oT, kmax2, s_scr, bu, bnat, cw):
    i = pl.program_id(0)

    @pl.when(i == 0)
    def _prologue():
        x = x_ref[...]
        k = _dg(x, wk_ref[...], NT).astype(BF16)
        kaug[...] = jnp.concatenate([k, jnp.ones((S, DH), BF16)], axis=1)
        kf = k.astype(F32)
        kn = jnp.max(jnp.sum(kf * kf, axis=1, keepdims=True), axis=0, keepdims=True)
        kmax2[...] = jnp.broadcast_to(kn, (8, 128))
        vt = _dg(wv_ref[...], x, NT).astype(BF16)
        for c in range(NKC):
            vT[c] = vt[:, c * KC:(c + 1) * KC]
        wqT[...] = wq_ref[...].T

        lre = lre_ref[...].astype(F32).reshape(1, D)
        lim = lim_ref[...].astype(F32).reshape(1, D)
        dt = jnp.exp(ldt_ref[...].astype(F32).reshape(1, D)).astype(BF16).astype(F32)
        mag = jnp.exp(dt * lre)
        ar = mag * jnp.cos(dt * lim)
        ai = mag * jnp.sin(dt * lim)
        den = lre * lre + lim * lim
        nr, ni = ar - 1.0, ai
        cr = (nr * lre + ni * lim) / den
        ci = (ni * lre - nr * lim) / den
        c_re = cre_ref[...].astype(F32)
        c_im = cim_ref[...].astype(F32)
        cw[0] = (2.0 * (c_re * cr - c_im * ci)).astype(BF16)
        cw[1] = (-2.0 * (c_re * ci + c_im * cr)).astype(BF16)

        for ri, b_ref in enumerate((bre_ref, bim_ref)):
            for j in range(NSEG):
                t = _dg(x_ref[j * SEGL:(j + 1) * SEGL, :], b_ref[...], NT)
                for c in range(LT):
                    bu[ri * LT + c, pl.ds(j * PITCH, SEGL), :] = t[:, c * 128:(c + 1) * 128]

        ars = [jnp.broadcast_to(ar[:, c * 128:(c + 1) * 128], (NSEG, 128)) for c in range(LT)]
        ais = [jnp.broadcast_to(ai[:, c * 128:(c + 1) * 128], (NSEG, 128)) for c in range(LT)]

        def step(s, hr, hi):
            nhr, nhi = [], []
            for c in range(LT):
                br = bu[c, pl.ds(s, NSEG, stride=PITCH), :]
                bi = bu[LT + c, pl.ds(s, NSEG, stride=PITCH), :]
                nhr.append(ars[c] * hr[c] - ais[c] * hi[c] + br)
                nhi.append(ars[c] * hi[c] + ais[c] * hr[c] + bi)
            return nhr, nhi

        zero = jnp.zeros((NSEG, 128), F32)
        hr, hi = [zero] * LT, [zero] * LT
        for s in range(SEGL):
            hr, hi = step(s, hr, hi)

        pr, pi = ars, ais
        for _ in range(7):
            sq = [_cmul(pr[c], pi[c], pr[c], pi[c]) for c in range(LT)]
            pr, pi = [t[0] for t in sq], [t[1] for t in sq]
        row = lax.broadcasted_iota(jnp.int32, (NSEG, 128), 0)
        sh = 1
        while sh < NSEG:
            nr_, ni_ = [], []
            for c in range(LT):
                sr = jnp.where(row >= sh, pltpu.roll(hr[c], sh, 0), 0.0)
                si = jnp.where(row >= sh, pltpu.roll(hi[c], sh, 0), 0.0)
                mr, mi = _cmul(pr[c], pi[c], sr, si)
                nr_.append(hr[c] + mr)
                ni_.append(hi[c] + mi)
            hr, hi = nr_, ni_
            sq = [_cmul(pr[c], pi[c], pr[c], pi[c]) for c in range(LT)]
            pr, pi = [t[0] for t in sq], [t[1] for t in sq]
            sh *= 2
        hr = [jnp.where(row >= 1, pltpu.roll(t, 1, 0), 0.0) for t in hr]
        hi = [jnp.where(row >= 1, pltpu.roll(t, 1, 0), 0.0) for t in hi]

        SB = 8
        for sb in range(SEGL // SB):
            rows_r, rows_i = [], []
            for s in range(sb * SB, (sb + 1) * SB):
                hr, hi = step(s, hr, hi)
                rows_r.append(jnp.concatenate(hr, axis=1))
                rows_i.append(jnp.concatenate(hi, axis=1))
            hbr = jnp.concatenate(rows_r, axis=0).astype(BF16)
            hbi = jnp.concatenate(rows_i, axis=0).astype(BF16)
            y = _dg(hbr, cw[0], NT) + _dg(hbi, cw[1], NT)
            for u in range(SB):
                s = sb * SB + u
                for c in range(LT):
                    bnat[c, pl.ds(s, NSEG, stride=PITCH), :] = (
                        y[u * NSEG:(u + 1) * NSEG, c * 128:(c + 1) * 128])

    xb = x_ref[pl.ds(pl.multiple_of(i * QB, QB), QB), :]
    qt = (_dg(wqT[...], xb, NT) * (DH ** -0.5 * LOG2E)).astype(BF16)
    qf = qt.astype(F32)
    n2 = jnp.sum((qf * qf).reshape(H, DH, QB), axis=1, keepdims=True)
    km = jnp.tile(kmax2[0:1, :], (1, QB // 128))
    mh = jnp.sqrt(n2 * km[None]) * (-1.02 / DH)
    mt = jnp.broadcast_to(mh, (H, DH, QB)).reshape(H * DH, QB).astype(BF16)
    for h in range(H):
        qa[h * DA:h * DA + DH, :] = qt[h * DH:(h + 1) * DH, :]
        qa[h * DA + DH:(h + 1) * DA, :] = mt[h * DH:(h + 1) * DH, :]

    def fast_body(it, bad):
        items = [(j, c) for j in range(HU) for c in range(NKC)]
        qs, accs, ls, ps = {}, {}, {}, {}
        for n in range(len(items) + DLY):
            if n < len(items):
                j, c = items[n]
                if c == 0:
                    h = it * HU + j
                    qs[j] = qa[pl.ds(pl.multiple_of(h * DA, DA), DA), :]
                s = _dot(kaug[c * KC:(c + 1) * KC, :], qs[j])
                p = jnp.exp2(s)
                ll = p.reshape(KC // 8, 8, QB).sum(axis=0)
                ls[j] = ll if c == 0 else ls[j] + ll
                ps[n] = p.astype(BF16)
            if n >= DLY:
                j, c = items[n - DLY]
                o = _dot(vT[c], ps.pop(n - DLY))
                accs[j] = o if c == 0 else accs[j] + o
                if c == NKC - 1:
                    h = it * HU + j
                    l = jnp.sum(ls[j], axis=0, keepdims=True)
                    ok = jnp.logical_and(l > 2.0 ** -80, l < 2.0 ** 80)
                    bad = jnp.maximum(bad, jnp.where(ok, 0.0, 1.0))
                    oT[pl.ds(pl.multiple_of(h * DH, DH), DH), :] = (accs[j] / l).astype(BF16)
        return bad

    bad = lax.fori_loop(0, H // HU, fast_body, jnp.zeros((1, QB), F32))

    @pl.when(jnp.max(bad) > 0.0)
    def _exact():
        def head(h, carry):
            q = qa[pl.ds(pl.multiple_of(h * DA, DA), DH), :]

            def p1(c, m):
                r = pl.ds(pl.multiple_of(c * KC, KC), KC)
                s = _dot(kaug[r, 0:DH], q)
                s_scr[r, :] = s
                return jnp.maximum(m, jnp.max(s, axis=0, keepdims=True))

            m = lax.fori_loop(0, NKC, p1, jnp.full((1, QB), -jnp.inf, F32))

            def p2(c, carry2):
                acc, l = carry2
                r = pl.ds(pl.multiple_of(c * KC, KC), KC)
                p = jnp.exp2(s_scr[r, :] - m)
                return (acc + _dot(vT[c], p.astype(BF16)),
                        l + jnp.sum(p, axis=0, keepdims=True))

            acc, l = lax.fori_loop(0, NKC, p2,
                                   (jnp.zeros((DH, QB), F32), jnp.zeros((1, QB), F32)))
            oT[pl.ds(pl.multiple_of(h * DH, DH), DH), :] = (acc / l).astype(BF16)
            return carry

        lax.fori_loop(0, H, head, 0)

    a = _dg(oT[...], wo_ref[...], TN)
    xf = xb.astype(F32)
    gw = gw_ref[...].astype(F32).reshape(1, D)
    g = jax.nn.sigmoid(jnp.sum(xf * gw, axis=1, keepdims=True))
    dsk = dsk_ref[...].astype(F32).reshape(1, D)
    for u in range(QB // SEGL):
        j = i * (QB // SEGL) + u
        b = jnp.concatenate([bnat[c, pl.ds(j * PITCH, SEGL), :] for c in range(LT)], axis=1)
        r = slice(u * SEGL, (u + 1) * SEGL)
        b = b + xf[r] * dsk
        out_ref[r, :] = g[r] * a[r] + (1.0 - g[r]) * b


@jax.jit
def pallas_gated_mix__grouped_kv_mqa__ssm_conv_s5__prompt_kernel(
        A_x, A_wq, A_wk, A_wv, A_wo, B_x, B_Lambda_re, B_Lambda_im, B_B_re, B_B_im,
        B_C_re, B_C_im, B_log_dt, B_Dskip, gate_w):
    del B_x
    x = A_x.reshape(S, D)
    full2 = lambda shape: pl.BlockSpec(shape, lambda i: (0, 0))
    full1 = pl.BlockSpec((D,), lambda i: (0,))
    out = pl.pallas_call(
        _kernel,
        grid=(NQB,),
        in_specs=[full2((S, D)), full2((D, D)), full2((DH, D)), full2((DH, D)), full2((D, D)),
                  full1, full1, full2((D, D)), full2((D, D)), full2((D, D)), full2((D, D)),
                  full1, full1, full1],
        out_specs=pl.BlockSpec((QB, D), lambda i: (i, 0)),
        out_shape=jax.ShapeDtypeStruct((S, D), F32),
        scratch_shapes=[
            pltpu.VMEM((S, DA), BF16),
            pltpu.VMEM((NKC, DH, KC), BF16),
            pltpu.VMEM((D, D), BF16),
            pltpu.VMEM((H * DA, QB), BF16),
            pltpu.VMEM((H * DH, QB), BF16),
            pltpu.VMEM((8, 128), F32),
            pltpu.VMEM((S, QB), F32),
            pltpu.VMEM((2 * LT, NSEG * PITCH, 128), F32),
            pltpu.VMEM((LT, NSEG * PITCH, 128), F32),
            pltpu.VMEM((2, D, D), BF16),
        ],
        compiler_params=pltpu.CompilerParams(
            dimension_semantics=("arbitrary",), vmem_limit_bytes=100 * 1024 * 1024),
        name="gm_kernel",
    )(x, A_wq, A_wk.T, A_wv.T, A_wo, B_Lambda_re, B_Lambda_im, B_B_re, B_B_im,
      B_C_re, B_C_im, B_log_dt, B_Dskip, gate_w)
    return out.reshape(1, S, D)
```

```python
import jax
import jax.numpy as jnp
from jax import lax
import jax.experimental.pallas as pl
import jax.experimental.pallas.tpu as pltpu

S, D, H, DH = 2048, 512, 32, 16
DA = 2 * DH
DF = 24
QB, KC = 512, 128
NQB, NKC = S // QB, S // KC
R = 16
KM = KC - R
NSEG, SEGL, PITCH = 16, 128, 129
SROWS = (NSEG + 1) * PITCH + 7 - ((NSEG + 1) * PITCH + 7) % 8
LT = D // 128
HU = 8
AOFF = 64
XA = 128
SB = 16
SERD = 13
LOG2E = 1.4426950408889634
F32, BF16, I32 = jnp.float32, jnp.bfloat16, jnp.int32

NT = (((1,), (1,)), ((), ()))
TN = (((0,), (0,)), ((), ()))


def _dot(a, b):
    return jnp.dot(a, b, preferred_element_type=F32)


def _dg(a, b, dims):
    return lax.dot_general(a, b, dims, preferred_element_type=F32)


def _cmul(ar, ai, br, bi):
    return ar * br - ai * bi, ar * bi + ai * br


def _kernel(x_hbm, wq_hbm, wk_hbm, wv_hbm, wo_hbm, lre_hbm, lim_hbm, bre_hbm, bim_hbm,
            cre_hbm, cim_hbm, ldt_hbm, dsk_hbm, gw_hbm, out_hbm,
            x_v, wq_v, wkv_v, wo_v, lre_v, lim_v, bre_v, bim_v, cre_v, cim_v, ldt_v, dsk_v, gw_v,
            sems, osems, obuf,
            klhs, vT, kb, wqT, qa, qf, kmx_s, zbuf, oT, s_scr, bu, bnat, cw):
    i = pl.program_id(0)

    @pl.when(i == 0)
    def _prologue():
        zbuf[...] = jnp.zeros(zbuf.shape, F32)
        def cp(src, dst, n):
            return pltpu.make_async_copy(src, dst, sems.at[n])
        cps = {
            "xa": cp(x_hbm.at[pl.ds(0, XA)], x_v.at[pl.ds(0, XA)], 17),
            "bre": cp(bre_hbm, bre_v, 10),
            "x0": cp(x_hbm.at[pl.ds(XA, QB - XA)], x_v.at[pl.ds(XA, QB - XA)], 3),
            "bim": cp(bim_hbm, bim_v, 11),
            "x1": cp(x_hbm.at[pl.ds(QB, QB)], x_v.at[pl.ds(QB, QB)], 7),
            "x2": cp(x_hbm.at[pl.ds(2 * QB, QB)], x_v.at[pl.ds(2 * QB, QB)], 8),
            "x3": cp(x_hbm.at[pl.ds(3 * QB, QB)], x_v.at[pl.ds(3 * QB, QB)], 9),
            "lre": cp(lre_hbm, lre_v, 4),
            "lim": cp(lim_hbm, lim_v, 5),
            "ldt": cp(ldt_hbm, ldt_v, 6),
            "wq": cp(wq_hbm, wq_v, 0),
            "wk": cp(wk_hbm, wkv_v.at[0], 1),
            "wv": cp(wv_hbm, wkv_v.at[1], 2),
            "cre": cp(cre_hbm, cre_v, 12),
            "cim": cp(cim_hbm, cim_v, 13),
            "wo": cp(wo_hbm, wo_v, 14),
            "dsk": cp(dsk_hbm, dsk_v, 15),
            "gw": cp(gw_hbm, gw_v, 16),
        }
        for c_ in cps.values():
            c_.start()

        def wait(*names):
            for nm in names:
                if nm in cps:
                    cps.pop(nm).wait()

        def bu_rows(ri, j):
            b_ref = (bre_v, bim_v)[ri]
            t = _dg(x_v[j * SEGL:(j + 1) * SEGL, :], b_ref[...], NT)
            for c in range(LT):
                bu[ri * LT + c, pl.ds(j * PITCH, SEGL), :] = t[:, c * 128:(c + 1) * 128]

        J0 = QB // SEGL
        wait("xa", "bre")
        for j in range(J0):
            if j * SEGL == XA:
                wait("x0")
            bu_rows(0, j)
        wait("bim")
        for j in range(J0):
            bu_rows(1, j)
        wait("x1", "x2", "x3")

        def prep():
            wait("wq", "wk", "wv", "lre", "lim", "ldt", "cre", "cim", "wo", "dsk", "gw")
            wqT[0:D, :] = wq_v[...].T
            wqT[D:D + DH, :] = wkv_v[0]
            wqT[D + DH:D + 2 * DH, :] = wkv_v[1]

            lre = lre_v[...].astype(F32).reshape(1, D)
            lim = lim_v[...].astype(F32).reshape(1, D)
            dt = jnp.exp(ldt_v[...].astype(F32).reshape(1, D)).astype(BF16).astype(F32)
            mag = jnp.exp(dt * lre)
            ar = mag * jnp.cos(dt * lim)
            ai = mag * jnp.sin(dt * lim)
            den = lre * lre + lim * lim
            nr, ni = ar - 1.0, ai
            cr = (nr * lre + ni * lim) / den
            ci = (ni * lre - nr * lim) / den

            c_re = cre_v[...].astype(F32)
            c_im = cim_v[...].astype(F32)
            cw[0] = (2.0 * (c_re * cr - c_im * ci)).astype(BF16)
            cw[1] = (-2.0 * (c_re * ci + c_im * cr)).astype(BF16)

            return ar, ai

        for j in range(J0, NSEG):
            bu_rows(0, j)
        ar, ai = prep()
        for j in range(J0, NSEG):
            bu_rows(1, j)

        def qkv_dot(b):
            return _dg(wqT[...], x_v[b * QB:(b + 1) * QB, :], NT)

        def qkv_post(b, t):
            cols = slice(b * QB, (b + 1) * QB)
            for h in range(H):
                qt = (t[h * DH:(h + 1) * DH] * (DH ** -0.5 * LOG2E)).astype(BF16)
                qv = qt.astype(F32)
                n2 = jnp.sum(qv * qv, axis=0, keepdims=True)
                mt = jnp.broadcast_to(jnp.sqrt(n2) * (-1.0 / DH), (DH, QB)).astype(BF16)
                m8 = mt[0:8].astype(F32) * float(DH)
                qa[h * DA:h * DA + DH, cols] = qt
                qa[h * DA + DH:(h + 1) * DA, cols] = mt
                qf[h * DF:h * DF + DH, cols] = qv
                qf[h * DF + DH:(h + 1) * DF, cols] = m8
            kt = t[D:D + DH].astype(BF16).astype(F32)
            kn = jnp.max(jnp.sum(kt * kt, axis=0, keepdims=True), axis=1, keepdims=True)
            ka = jnp.concatenate([kt, jnp.zeros((128 - DH, QB), F32)], axis=0).T
            vt = pltpu.bitcast(t[D + DH:D + 2 * DH].astype(BF16), I32)
            for cc in range(QB // KC):
                c = b * (QB // KC) + cc
                kw = pltpu.bitcast(ka[cc * KC:(cc + 1) * KC].astype(BF16), I32)
                klhs[c * (KM // 2):(c + 1) * (KM // 2), :] = kw[0:KM // 2]
                klhs[(NKC * KM + c * R) // 2:(NKC * KM + (c + 1) * R) // 2, :] = kw[KM // 2:KC // 2]
                vT[c] = vt[:, cc * KC:(cc + 1) * KC]
                kr = ka[cc * KC + KM:(cc + 1) * KC]
                for d in range(DH):
                    kb[c, d] = jnp.broadcast_to(kr[:, d:d + 1], (R, 128))
            return kn

        ars = [jnp.broadcast_to(ar[:, c * 128:(c + 1) * 128], (NSEG, 128)) for c in range(LT)]
        ais = [jnp.broadcast_to(ai[:, c * 128:(c + 1) * 128], (NSEG, 128)) for c in range(LT)]

        def step(s, hr, hi):
            nhr, nhi = [], []
            for c in range(LT):
                br = bu[c, pl.ds(s, NSEG, stride=PITCH), :]
                bi = bu[LT + c, pl.ds(s, NSEG, stride=PITCH), :]
                nhr.append(ars[c] * hr[c] - ais[c] * hi[c] + br)
                nhi.append(ars[c] * hi[c] + ais[c] * hr[c] + bi)
            return nhr, nhi

        zero = jnp.zeros((NSEG, 128), F32)
        hr, hi = [zero] * LT, [zero] * LT
        kn = qkv_post(0, qkv_dot(0))
        for s in range(SEGL // 2):
            hr, hi = step(s, hr, hi)
        kn = jnp.maximum(kn, qkv_post(1, qkv_dot(1)))
        for s in range(SEGL // 2, SEGL):
            hr, hi = step(s, hr, hi)
        kn = jnp.maximum(kn, qkv_post(2, qkv_dot(2)))

        pr, pi = ars, ais
        for _ in range(7):
            sq = [_cmul(pr[c], pi[c], pr[c], pi[c]) for c in range(LT)]
            pr, pi = [t[0] for t in sq], [t[1] for t in sq]
        row = lax.broadcasted_iota(I32, (NSEG, 128), 0)
        sh = 1
        while sh < NSEG:
            nr_, ni_ = [], []
            for c in range(LT):
                mr, mi = _cmul(pr[c], pi[c], pltpu.roll(hr[c], sh, 0), pltpu.roll(hi[c], sh, 0))
                nr_.append(hr[c] + jnp.where(row >= sh, mr, 0.0))
                ni_.append(hi[c] + jnp.where(row >= sh, mi, 0.0))
            hr, hi = nr_, ni_
            sq = [_cmul(pr[c], pi[c], pr[c], pi[c]) for c in range(LT)]
            pr, pi = [t[0] for t in sq], [t[1] for t in sq]
            sh *= 2
        hr = [jnp.where(row >= 1, pltpu.roll(t, 1, 0), 0.0) for t in hr]
        hi = [jnp.where(row >= 1, pltpu.roll(t, 1, 0), 0.0) for t in hi]

        kn = jnp.maximum(kn, qkv_post(3, qkv_dot(3)))

        kmx = (jnp.sqrt(kn) * 1.02).astype(BF16)
        kmxf = jnp.broadcast_to(kmx.astype(F32), (8, 128))
        kmx_s[...] = kmxf
        lane = lax.broadcasted_iota(I32, (8, 128), 1)
        kword = pltpu.bitcast(jnp.broadcast_to(kmx, (16, 128)), I32)
        msk = jnp.logical_and(lane >= DH, lane < DA)
        for r0 in range(0, NKC * KM // 2, 8):
            klhs[r0:r0 + 8, :] = jnp.where(msk, kword, klhs[r0:r0 + 8, :])

        for sb in range(SEGL // SB):
            rows_r, rows_i = [], []
            for s in range(sb * SB, (sb + 1) * SB):
                hr, hi = step(s, hr, hi)
                rows_r.append(jnp.concatenate(hr, axis=1))
                rows_i.append(jnp.concatenate(hi, axis=1))
            hbr = jnp.concatenate(rows_r, axis=0).astype(BF16)
            hbi = jnp.concatenate(rows_i, axis=0).astype(BF16)
            y = _dg(hbr, cw[0], NT) + _dg(hbi, cw[1], NT)
            for u in range(SB):
                s = sb * SB + u
                for c in range(LT):
                    bnat[c, pl.ds(s, NSEG, stride=PITCH), :] = (
                        y[u * NSEG:(u + 1) * NSEG, c * 128:(c + 1) * 128])
        assert not cps

    qcols = pl.ds(pl.multiple_of(i * QB, QB), QB)
    NU = QB // SEGL

    def out_copy(step, u):
        slot = step % 2
        rows = pl.ds(pl.multiple_of((step * NU + u) * SEGL, SEGL), SEGL)
        return pltpu.make_async_copy(obuf.at[slot, pl.ds(u * SEGL, SEGL)], out_hbm.at[rows],
                                     osems.at[slot, u])

    @pl.when(i >= 2)
    def _():
        for u in range(NU):
            out_copy(i - 2, u).wait()

    def pv(c, p):
        return _dot(pltpu.bitcast(vT[c], BF16), p)

    def fast_body(it, lstat):
        qs, qfh, mneg, accs, ls, head_p = {}, {}, {}, {}, {}, {}
        prev, pend, lstat = [None], [], [lstat]

        def scores(j, lo, hi):
            kl = pltpu.bitcast(klhs[lo // 2:hi // 2, :], BF16)
            p = jnp.exp2(_dot(kl[:, 0:DA], qs[j]))
            addl(j, p)
            return p

        def addl(j, p):
            for r0 in range(0, p.shape[0], 8):
                ls[j] = p[r0:r0 + 8] if j not in ls else ls[j] + p[r0:r0 + 8]

        def vpu_scores(j, c):
            tiles = []
            for t in range(QB // 128):
                sv = mneg[j][t]
                if prev[0] is not None:
                    sv = jnp.where(prev[0] > jnp.inf, prev[0], sv)
                for d in range(DH):
                    sv = sv + kb[c, d] * jnp.broadcast_to(qfh[j][t][d:d + 1], (R, 128))
                    if d == SERD - 1:
                        prev[0] = sv
                tiles.append(sv)
            p = jnp.exp2(jnp.concatenate(tiles, axis=1))
            addl(j, p)
            return p

        def do_v(j, c, p):
            accs[j] = (zbuf[...] if c == 0 else accs[j]) + pv(c, p)
            if c == NKC - 1:
                l = jnp.sum(ls[j], axis=0, keepdims=True)
                rows = pl.ds(pl.multiple_of((it * HU + j) * DH, DH), DH)
                oT[rows, :] = (accs[j] * (1.0 / l)).astype(BF16)
                lstat[0] = (lstat[0][0] + l, jnp.minimum(lstat[0][1], l))

        for j in range(HU):
            h = it * HU + j
            qs[j] = qa[pl.ds(pl.multiple_of(h * DA, DA), DA), qcols]
            qq = qf[pl.ds(pl.multiple_of(h * DF, 8), DF), qcols]
            qfh[j] = [qq[:, t * 128:(t + 1) * 128] for t in range(QB // 128)]
            mneg[j] = [jnp.concatenate([qfh[j][t][DH:DF] * kmx_s[...]] * (R // 8), axis=0)
                       for t in range(QB // 128)]
            head_p[0] = scores(j, 0, AOFF)
            for c in range(NKC):
                p = scores(j, c * KM + AOFF, min((c + 1) * KM + AOFF, NKC * KM))
                parts = [head_p.pop(c), p[0:KM - AOFF], vpu_scores(j, c)]
                if c < NKC - 1:
                    head_p[c + 1] = p[KM - AOFF:KM]
                pend.append((j, c, jnp.concatenate(parts, axis=0)))
                if len(pend) > 1:
                    do_v(*pend.pop(0))
        do_v(*pend.pop(0))
        return lstat[0]

    lsum, lmin = lax.fori_loop(0, H // HU, fast_body,
                               (jnp.zeros((1, QB), F32), jnp.ones((1, QB), F32)))
    bad = jnp.where(jnp.logical_and(lsum < 2.0 ** 90, lmin > 2.0 ** -80), 0.0, 1.0)

    @pl.when(jnp.max(bad) > 0.0)
    def _exact():
        def head(h, carry):
            q = qa[pl.ds(pl.multiple_of(h * DA, DA), DH), qcols]

            def p1(c, m):
                kl = pltpu.bitcast(jnp.concatenate(
                    [klhs[pl.ds(pl.multiple_of(c * (KM // 2), 8), KM // 2), :],
                     klhs[pl.ds(pl.multiple_of((NKC * KM) // 2 + c * (R // 2), 8), R // 2), :]],
                    axis=0), BF16)
                s = _dot(kl[:, 0:DH], q)
                s_scr[pl.ds(pl.multiple_of(c * KC, KC), KC), :] = s
                return jnp.maximum(m, jnp.max(s, axis=0, keepdims=True))

            m = lax.fori_loop(0, NKC, p1, jnp.full((1, QB), -jnp.inf, F32))

            def p2(c, carry2):
                acc, l = carry2
                p = jnp.exp2(s_scr[pl.ds(pl.multiple_of(c * KC, KC), KC), :] - m)
                return (acc + pv(c, p.astype(BF16)),
                        l + jnp.sum(p, axis=0, keepdims=True))

            acc, l = lax.fori_loop(0, NKC, p2,
                                   (jnp.zeros((DH, QB), F32), jnp.zeros((1, QB), F32)))
            oT[pl.ds(pl.multiple_of(h * DH, DH), DH), :] = (acc / l).astype(BF16)
            return carry

        lax.fori_loop(0, H, head, 0)

    gw = gw_v[...].astype(F32).reshape(1, D)
    dsk = dsk_v[...].astype(F32).reshape(1, D)
    for u in range(NU):
        j = i * NU + u
        r = slice(u * SEGL, (u + 1) * SEGL)
        a = _dg(oT[:, r], wo_v[...], TN)
        xf = x_v[pl.ds(pl.multiple_of(j * SEGL, SEGL), SEGL), :].astype(F32)
        g = jax.nn.sigmoid(jnp.sum(xf * gw, axis=1, keepdims=True))
        b = jnp.concatenate([bnat[c, pl.ds(j * PITCH, SEGL), :] for c in range(LT)], axis=1)
        b = b + xf * dsk
        obuf[i % 2, r, :] = g * a + (1.0 - g) * b
        out_copy(i, u).start()

    @pl.when(i == NQB - 1)
    def _():
        for u in range(NU):
            out_copy(i - 1, u).wait()
        for u in range(NU):
            out_copy(i, u).wait()


@jax.jit
def pallas_gated_mix__grouped_kv_mqa__ssm_conv_s5__prompt_kernel(
        A_x, A_wq, A_wk, A_wv, A_wo, B_x, B_Lambda_re, B_Lambda_im, B_B_re, B_B_im,
        B_C_re, B_C_im, B_log_dt, B_Dskip, gate_w):
    del B_x
    x = A_x.reshape(S, D)
    hbm = pl.BlockSpec(memory_space=pl.ANY)
    vec = pltpu.VMEM((D,), BF16)
    mat = pltpu.VMEM((D, D), BF16)
    out = pl.pallas_call(
        _kernel,
        grid=(NQB,),
        in_specs=[hbm] * 14,
        out_specs=hbm,
        out_shape=jax.ShapeDtypeStruct((S, D), F32),
        scratch_shapes=[
            pltpu.VMEM((S, D), BF16),
            mat,
            pltpu.VMEM((2, DH, D), BF16),
            mat,
            vec, vec,
            mat, mat, mat, mat,
            vec, vec, vec,
            pltpu.SemaphoreType.DMA((18,)),
            pltpu.SemaphoreType.DMA((2, QB // SEGL)),
            pltpu.VMEM((2, QB, D), F32),
            pltpu.VMEM((S // 2, 128), I32),
            pltpu.VMEM((NKC, DH // 2, KC), I32),
            pltpu.VMEM((NKC, DH, R, 128), F32),
            pltpu.VMEM((D + 2 * DH, D), BF16),
            pltpu.VMEM((H * DA, S), BF16),
            pltpu.VMEM((H * DF, S), F32),
            pltpu.VMEM((8, 128), F32),
            pltpu.VMEM((DH, QB), F32),
            pltpu.VMEM((H * DH, QB), BF16),
            pltpu.VMEM((S, QB), F32),
            pltpu.VMEM((2 * LT, SROWS, 128), F32),
            pltpu.VMEM((LT, SROWS, 128), F32),
            pltpu.VMEM((2, D, D), BF16),
        ],
        compiler_params=pltpu.CompilerParams(
            dimension_semantics=("arbitrary",), vmem_limit_bytes=100 * 1024 * 1024),
        name="gm_kernel",
    )(x, A_wq, A_wk.T, A_wv.T, A_wo, B_Lambda_re, B_Lambda_im, B_B_re, B_B_im,
      B_C_re, B_C_im, B_log_dt, B_Dskip, gate_w)
    return out.reshape(1, S, D)
```
